```python
import os as _os
_os.environ.setdefault("JAX_PLATFORMS", "cpu")
import jax
import jax.numpy as jnp

def _softmax(x, axis=-1):
    return jax.nn.softmax(x, axis=axis)
def _gelu(x):
    return jax.nn.gelu(x, approximate=True)
def _silu(x):
    return jax.nn.silu(x)
def _sigmoid(x):
    return jax.nn.sigmoid(x)
def _layernorm(x, axis=-1, eps=1e-5):
    m = jnp.mean(x, axis=axis, keepdims=True)
    v = jnp.var(x, axis=axis, keepdims=True)
    return (x - m) / jnp.sqrt(v + eps)
def _scatter_add(tgt, idx, src, axis=0):
    return tgt.at[idx].add(src)
def _segment_sum(src, seg, n):
    return jax.ops.segment_sum(src, seg, n)
class _Rng:
    def __init__(self, key):
        self._k = key
    def _next(self):
        self._k, sub = jax.random.split(self._k)
        return sub
    def normal(self, shape):
        return jax.random.normal(self._next(), shape, dtype=jnp.bfloat16)
    def randint(self, lo, hi, shape):
        return jax.random.randint(self._next(), shape, lo, hi, dtype=jnp.int32)
    def uniform(self, shape, lo=0.0, hi=1.0):
        return jax.random.uniform(self._next(), shape, jnp.bfloat16, lo, hi)
    def permutation(self, n):
        return jax.random.permutation(self._next(), n)


kernel_name = 'parallel_sum__sliding_block__moe_arch_mod__prompt'

def setup_inputs():
    _rng = _Rng(jax.random.key(int.from_bytes(__import__("os").urandom(4), "little")))
    _w = (lambda a: (lambda t: t.astype(jnp.bfloat16) if jnp.issubdtype(t.dtype, jnp.floating) else t)(jnp.asarray(a)))
    def _A_setup():
        B, S, D = 1, 2048, 512
        return {
            "x": _w((lambda *s: _rng.normal(s) * 0.05)(B, S, D)),
            "wqkv": _w((lambda *s: _rng.normal(s) * 0.05)(D, 3 * D)),
            "wo": _w((lambda *s: _rng.normal(s) * 0.05)(D, D)),
        }
    _A_in = _A_setup()

    def _B_setup():
        B, S, D, F, C = 1, 2048, 512, 1376, 1
        return {
            "x": _w((lambda *s: _rng.normal(s) * 0.05)(B, S, D)),
            "w_r": _w((lambda *s: _rng.normal(s) * 0.05)(D)),
            "w_gate": _w((lambda *s: _rng.normal(s) * 0.05)(D, F)),
            "w_up": _w((lambda *s: _rng.normal(s) * 0.05)(D, F)),
            "w_down": _w((lambda *s: _rng.normal(s) * 0.05)(F, D)),
        }
    _B_in = _B_setup()

    return {
        "A_x": _A_in["x"],
        "A_wqkv": _A_in["wqkv"],
        "A_wo": _A_in["wo"],
        "B_x": _B_in["x"],
        "B_w_r": _B_in["w_r"],
        "B_w_gate": _B_in["w_gate"],
        "B_w_up": _B_in["w_up"],
        "B_w_down": _B_in["w_down"],
    }

def reference(A_x, A_wqkv, A_wo, B_x, B_w_r, B_w_gate, B_w_up, B_w_down):
    def _A_ref(x, wqkv, wo):
        B, S, D = x.shape
        H = 32; Dh = D // H; W = 256
        qkv = (lambda x, *d: x.transpose(*d))((x @ wqkv).reshape(B, S, 3, H, Dh), 2, 0, 3, 1, 4)
        q, k, v = qkv[0], qkv[1], qkv[2]
        scores = jnp.einsum("bhqd,bhkd->bhqk", q, k) * (Dh ** -0.5)
        idx = jnp.arange(S)
        mask = (idx[:, None] - idx[None, :] >= 0) & (idx[:, None] - idx[None, :] < W)
        scores = jnp.where(mask[None, None], scores, -1e9)
        p = _softmax(scores, axis=-1)
        o = jnp.einsum("bhqk,bhkd->bhqd", p, v)
        return (lambda x, *d: x.transpose(*d))(o, 0, 2, 1, 3).reshape(B, S, D) @ wo

    def _B_ref(x, w_r, w_gate, w_up, w_down):
        B, S, D = x.shape
        C = 1
        r = x @ w_r
        idx = jnp.argsort(-r, axis=-1)[:, :C]
        idx_e = jnp.repeat(idx.reshape(B, C, 1), D, axis=2)
        x_sel = jnp.take_along_axis(x, idx_e, axis=1)
        g = _silu(x_sel @ w_gate)
        u = x_sel @ w_up
        y = (g * u) @ w_down
        r_sel = _sigmoid(jnp.take_along_axis(r, idx, axis=1))
        y = y * r_sel.reshape(B, C, 1)
        b_off = (jnp.arange(B) * S).reshape(B, 1)
        flat_idx = (idx + b_off).reshape(B * C)
        zero = (x * 0.0).reshape(B * S, D)
        upd = _scatter_add(zero, flat_idx, y.reshape(B * C, D), axis=0)
        return x + upd.reshape(B, S, D)

    x = A_x
    xn = _layernorm(x, axis=-1)
    return x + _A_ref(xn, A_wqkv, A_wo) + _B_ref(xn, B_w_r, B_w_gate, B_w_up, B_w_down)
```

```python
import jax
import jax.numpy as jnp
from jax import lax
import jax.experimental.pallas as pl
import jax.experimental.pallas.tpu as pltpu

_S = 2048; _D = 512; _H = 32; _DH = 16; _W = 256; _F = 1376
_EPS = 1e-5
_CH = 256
_QB = 64
_KW = _W + _QB
_SB = 128
_NEG = -1e9
_LOG2E = 1.4426950408889634
_F32 = jnp.float32
_BF16 = jnp.bfloat16
_U32 = jnp.uint32
_NT = (((1,), (1,)), ((), ()))


def _bf16_round(v):
    return v.astype(_BF16).astype(_F32)


def _pack_rows(a):
    r, c = a.shape
    a4 = a.reshape(r // 16, 2, 8, c)
    lo = a4[:, 0].reshape(r // 2, c)
    hi = a4[:, 1].reshape(r // 2, c)
    return pltpu.pack_elementwise([lo, hi], packed_dtype=_BF16)


def _kernel(x_hbm, wqkv_hbm, wo_hbm, wr_ref, wgt_hbm, wut_hbm, wd_hbm,
            o_hbm,
            x_ref, wqkv_ref, wo_ref, wgt_ref, wut_ref, wd_ref, o_ref,
            xn_ref, xnp_ref, q_ref, k_ref, vt_ref, r_ref, wvt_ref, upd_ref,
            st_ref, m_ref, oblk_ref, sem_x, sem_w, sem_o):
    n_ch = _S // _CH

    def x_copy(c):
        rows = pl.ds(pl.multiple_of(c * _CH, _CH), _CH)
        return pltpu.make_async_copy(x_hbm.at[rows, :], x_ref.at[rows, :], sem_x.at[c])

    w_pairs = ((wqkv_hbm, wqkv_ref), (wo_hbm, wo_ref), (wgt_hbm, wgt_ref), (wut_hbm, wut_ref), (wd_hbm, wd_ref))

    def w_copy(i):
        return pltpu.make_async_copy(w_pairs[i][0], w_pairs[i][1], sem_w.at[i])

    def o_copy(sb):
        rows = pl.ds(pl.multiple_of(sb * _SB, _SB), _SB)
        return pltpu.make_async_copy(o_ref.at[rows, :], o_hbm.at[rows, :], sem_o)

    x_copy(0).start()
    w_copy(0).start()
    for c in range(1, n_ch):
        x_copy(c).start()

    k_ref[0:_W, :] = jnp.zeros((_W, _D), _BF16)
    vt_ref[:, 0:_W] = jnp.zeros((_D, _W), _BF16)
    wr = wr_ref[...].reshape(1, _D).astype(_F32)

    def ln_chunk(c, carry):
        rows = pl.ds(pl.multiple_of(c * _CH, _CH), _CH)
        x_copy(c).wait()
        x = x_ref[rows, :].astype(_F32)
        mean = jnp.mean(x, axis=-1, keepdims=True)
        xc = x - mean
        var = jnp.mean(xc * xc, axis=-1, keepdims=True)
        mean_b = _bf16_round(mean)
        var_b = _bf16_round(var)
        den = _bf16_round(jnp.sqrt(_bf16_round(var_b + _EPS)))
        d = _bf16_round(x - mean_b)
        xn = _bf16_round(d / den)
        xn_ref[rows, :] = xn.astype(_BF16)
        xnp_ref[rows, :] = pltpu.bitcast(_pack_rows(xn), _BF16)
        r = jnp.sum(xn * wr, axis=-1, keepdims=True)
        r_ref[rows, :] = _bf16_round(r)
        return carry

    lax.fori_loop(0, _S // _CH, ln_chunk, 0)

    for i in range(1, 5):
        w_copy(i).start()
    w_copy(0).wait()
    wvt_ref[...] = wqkv_ref[:, 2 * _D:3 * _D].T
    qscale = (_DH ** -0.5) * _LOG2E

    def proj_chunk(c, carry):
        start = pl.multiple_of(c * _CH, _CH)
        xn = xn_ref[pl.ds(start, _CH), :]
        qk = jnp.dot(xn, wqkv_ref[:, 0:2 * _D], preferred_element_type=_F32)
        q_ref[pl.ds(start, _CH), :] = (qk[:, 0:_D] * qscale).astype(_BF16)
        k_ref[pl.ds(start + _W, _CH), :] = qk[:, _D:2 * _D].astype(_BF16)
        vt = lax.dot_general(wvt_ref[...], xnp_ref[pl.ds(start, _CH), :], _NT, preferred_element_type=_F32)
        vt_ref[:, pl.ds(start + _W, _CH)] = vt.astype(_BF16)
        return carry

    lax.fori_loop(0, _S // _CH, proj_chunk, 0)

    rv = r_ref[...]
    rmax = jnp.max(rv, axis=0, keepdims=True)
    tok = lax.broadcasted_iota(jnp.int32, (_S, 1), 0)
    idx = jnp.min(jnp.where(rv == rmax, tok, _S))
    base = pl.multiple_of((idx // 16) * 16, 16)
    tile = xn_ref[pl.ds(base, 16), :]
    row16 = lax.broadcasted_iota(jnp.int32, (16, _D), 0)
    xsel = jnp.where(row16 == (idx - base), tile.astype(_F32), 0.0).astype(_BF16)
    w_copy(2).wait()
    w_copy(3).wait()
    w_copy(4).wait()
    w_copy(1).wait()
    gpre = _bf16_round(lax.dot_general(xsel, wgt_ref[...], _NT, preferred_element_type=_F32))
    gate = _bf16_round(gpre * jax.nn.sigmoid(gpre))
    up = _bf16_round(lax.dot_general(xsel, wut_ref[...], _NT, preferred_element_type=_F32))
    hmid = (gate * up).astype(_BF16)
    y = _bf16_round(jnp.dot(hmid, wd_ref[...], preferred_element_type=_F32))
    rsel = _bf16_round(jax.nn.sigmoid(rmax))
    y = _bf16_round(y * rsel)
    upd_ref[...] = jnp.sum(y, axis=0, keepdims=True)

    head_u = lax.broadcasted_iota(jnp.int32, (_QB // 2, 128), 1) // _DH
    lane_o = lax.broadcasted_iota(jnp.int32, (_QB, 128), 1)
    parity_even = ((lane_o // _DH) % 2) == 0
    e_row = lax.broadcasted_iota(jnp.int32, (_QB, 128), 0)
    e_col = lax.broadcasted_iota(jnp.int32, (_QB, 128), 1) % _QB
    top_ok = e_row > e_col
    out_row = lax.broadcasted_iota(jnp.int32, (_SB, _D), 0)
    f_row = lax.broadcasted_iota(jnp.int32, (_KW, 128), 0)
    lo_p = lax.broadcasted_iota(jnp.int32, (3 * _QB, 128), 1) < _QB
    lo_1 = lax.broadcasted_iota(jnp.int32, (1, 128), 1) < _QB
    n_sb = _S // _SB

    def stage_a(q_start, g, slot, general):
        lanes = slice(g * 128, (g + 1) * 128)
        for half in range(2):
            q0 = pl.multiple_of(q_start + half * _QB, _QB)
            kw = k_ref[pl.ds(q0, _KW), lanes]
            qtu = pltpu.bitcast(q_ref[pl.ds(q0, _QB), lanes], _U32)
            order = [0, 1, 2, 3, 4, 5, 6, 7] if half == 0 else [1, 0, 3, 2, 5, 4, 7, 6]
            qmod = pltpu.bitcast(
                jnp.concatenate([jnp.where(head_u == h, qtu, jnp.zeros_like(qtu)) for h in order], axis=0),
                _BF16)
            st = lax.dot_general(kw, qmod, _NT, preferred_element_type=_F32)
            cols = []
            for j in range(4):
                sj = st[:, 128 * j:128 * (j + 1)]
                top = jnp.where(top_ok, sj[0:_QB], _NEG)
                bot = jnp.where(top_ok, _NEG, sj[_W:_KW])
                sj = jnp.concatenate([top, sj[_QB:_W], bot], axis=0)
                if general:
                    sj = jnp.where(f_row >= _W - q0, sj, _NEG)
                cols.append(sj)
            st = jnp.concatenate(cols, axis=1)
            st_ref[2 * slot + half] = st
            m_ref[2 * slot + half] = jnp.max(st, axis=0, keepdims=True)

    def stage_b(q_start, g, slot):
        lanes = slice(g * 128, (g + 1) * 128)
        pads = []
        invs = []
        zu = jnp.zeros((_QB // 2, 8 * _QB), _U32)
        for half in range(2):
            st = st_ref[2 * slot + half]
            m = m_ref[2 * slot + half]
            p = jnp.exp2(st - m)
            l = jnp.sum(p, axis=0, keepdims=True)
            invs.append(1.0 / l)
            pu = _pack_rows(p)
            pads.append(jnp.concatenate([pu, zu] if half == 0 else [zu, pu], axis=0))
        vtw = vt_ref[lanes, pl.ds(q_start, _SB + _W)]
        ot = []
        for j in range(4):
            tl = slice(128 * j, 128 * (j + 1))
            e_t = pads[0][:, tl]
            o_t = pads[1][:, tl]
            ma = pltpu.bitcast(jnp.where(lo_p, e_t, o_t), _BF16)
            mb = pltpu.bitcast(jnp.where(lo_p, o_t, e_t), _BF16)
            inva = jnp.where(lo_1, invs[0][:, tl], invs[1][:, tl])
            invb = jnp.where(lo_1, invs[1][:, tl], invs[0][:, tl])
            ota = jnp.dot(vtw[32 * j:32 * j + 16, :], ma, preferred_element_type=_F32)
            otb = jnp.dot(vtw[32 * j + 16:32 * j + 32, :], mb, preferred_element_type=_F32)
            ot.append(ota * inva)
            ot.append(otb * invb)
        t = jnp.concatenate(ot, axis=0).T
        t_lo = t[0:_QB, :]
        t_hi = t[_QB:2 * _QB, :]
        o_e = jnp.where(parity_even, t_lo, t_hi)
        o_o = jnp.where(parity_even, t_hi, t_lo)
        oblk_new = jnp.concatenate([o_e, o_o], axis=0).astype(_BF16)
        return oblk_new

    def stage_c(sb):
        q_start = pl.multiple_of(sb * _SB, _SB)
        attn = jnp.dot(oblk_ref[...], wo_ref[...], preferred_element_type=_F32)
        rows = pl.ds(q_start, _SB)
        res = x_ref[rows, :].astype(_F32) + attn + xn_ref[rows, :].astype(_F32)
        res = res + jnp.where(out_row == (idx - q_start), upd_ref[...], 0.0)
        o_ref[rows, :] = res.astype(o_ref.dtype)

    def super_block(sb, general, do_c):
        q_start = pl.multiple_of(sb * _SB, _SB)
        if do_c:
            stage_c(sb - 1)
        tiles = []
        for g in range(4):
            if g < 3:
                stage_a(q_start, g + 1, (g + 1) % 2, general)
            else:
                nxt = pl.multiple_of(jnp.minimum(sb + 1, n_sb - 1) * _SB, _SB)
                stage_a(nxt, 0, 0, general)
            tiles.append(stage_b(q_start, g, g % 2))
        for g in range(4):
            oblk_ref[:, g * 128:(g + 1) * 128] = tiles[g]
        if do_c:
            o_copy(sb - 1).start()

    def main_body(sb, carry):
        super_block(sb, False, True)
        return carry

    stage_a(0, 0, 0, True)
    super_block(0, True, False)
    super_block(1, True, True)
    lax.fori_loop(2, n_sb, main_body, 0)
    stage_c(n_sb - 1)
    o_copy(n_sb - 1).start()
    for sb in range(n_sb):
        o_copy(sb).wait()


@jax.jit
def pallas_parallel_sum__sliding_block__moe_arch_mod__prompt_kernel(
    A_x, A_wqkv, A_wo, B_x, B_w_r, B_w_gate, B_w_up, B_w_down):
    del B_x
    B, S, D = A_x.shape
    x2 = A_x.reshape(S, D)
    any_spec = pl.BlockSpec(memory_space=pl.ANY)
    out = pl.pallas_call(
        _kernel,
        out_shape=jax.ShapeDtypeStruct((S, D), A_x.dtype),
        in_specs=[any_spec, any_spec, any_spec, pl.BlockSpec(memory_space=pltpu.VMEM),
                  any_spec, any_spec, any_spec],
        out_specs=any_spec,
        scratch_shapes=[
            pltpu.VMEM((_S, _D), _BF16),
            pltpu.VMEM((_D, 3 * _D), _BF16),
            pltpu.VMEM((_D, _D), _BF16),
            pltpu.VMEM((_F, _D), _BF16),
            pltpu.VMEM((_F, _D), _BF16),
            pltpu.VMEM((_F, _D), _BF16),
            pltpu.VMEM((_S, _D), _BF16),
            pltpu.VMEM((_S, _D), _BF16),
            pltpu.VMEM((_S, _D), _BF16),
            pltpu.VMEM((_S, _D), _BF16),
            pltpu.VMEM((_S + _W, _D), _BF16),
            pltpu.VMEM((_D, _S + _W), _BF16),
            pltpu.VMEM((_S, 1), _F32),
            pltpu.VMEM((_D, _D), _BF16),
            pltpu.VMEM((1, _D), _F32),
            pltpu.VMEM((4, _KW, 8 * _QB), _F32),
            pltpu.VMEM((4, 1, 8 * _QB), _F32),
            pltpu.VMEM((_SB, _D), _BF16),
            pltpu.SemaphoreType.DMA((_S // _CH,)),
            pltpu.SemaphoreType.DMA((5,)),
            pltpu.SemaphoreType.DMA(()),
        ],
        compiler_params=pltpu.CompilerParams(vmem_limit_bytes=100 * 1024 * 1024),
        name="fused_ln_attn_moe",
    )(x2, A_wqkv, A_wo, B_w_r, B_w_gate.T, B_w_up.T, B_w_down)
    return out.reshape(B, S, D)
```

```python
import jax
import jax.numpy as jnp
from jax import lax
import jax.experimental.pallas as pl
import jax.experimental.pallas.tpu as pltpu

_S = 2048
_D = 512
_DH = 16
_W = 256
_F = 1376
_EPS = 1e-5
_NEG = -1e9

_CH = 256
_QB = 64
_KW = _W + _QB
_SB = 128

_LOG2E = 1.4426950408889634
_F32 = jnp.float32
_BF16 = jnp.bfloat16
_U32 = jnp.uint32
_NT = (((1,), (1,)), ((), ()))


def _bf16_round(v):
    return v.astype(_BF16).astype(_F32)


def _pack_rows(a):
    r, c = a.shape
    a4 = a.reshape(r // 16, 2, 8, c)
    lo = a4[:, 0].reshape(r // 2, c)
    hi = a4[:, 1].reshape(r // 2, c)
    return pltpu.pack_elementwise([lo, hi], packed_dtype=_BF16)


def _kernel(x_hbm, wqkv_hbm, wo_hbm, wr_ref, wgt_hbm, wut_hbm, wd_hbm,
            o_hbm,
            x_ref, wqkv_ref, wo_ref, wgt_ref, wut_ref, wd_ref, o_ref,
            xn_ref, xnp_ref, q_ref, k_ref, vt_ref, r_ref, wvt_ref, upd_ref,
            st_ref, m_ref, oblk_ref, res_ref, sem_x, sem_w, sem_o):
    n_ch = _S // _CH
    n_sb = _S // _SB

    def x_copy(c):
        rows = pl.ds(pl.multiple_of(c * _CH, _CH), _CH)
        return pltpu.make_async_copy(x_hbm.at[rows, :], x_ref.at[rows, :], sem_x.at[c])

    w_pairs = ((wqkv_hbm, wqkv_ref), (wo_hbm, wo_ref), (wgt_hbm, wgt_ref),
               (wut_hbm, wut_ref), (wd_hbm, wd_ref))

    def w_copy(i):
        return pltpu.make_async_copy(w_pairs[i][0], w_pairs[i][1], sem_w.at[i])

    def o_copy(sb):
        rows = pl.ds(pl.multiple_of(sb * _SB, _SB), _SB)
        return pltpu.make_async_copy(o_ref.at[rows, :], o_hbm.at[rows, :], sem_o)

    x_copy(0).start()
    w_copy(0).start()
    for c in range(1, n_ch):
        x_copy(c).start()

    k_ref[0:_W, :] = jnp.zeros((_W, _D), _BF16)
    vt_ref[:, 0:_W] = jnp.zeros((_D, _W), _BF16)
    wr = wr_ref[...].reshape(1, _D).astype(_F32)

    def ln_chunk(c, carry):
        rows = pl.ds(pl.multiple_of(c * _CH, _CH), _CH)
        x_copy(c).wait()
        x = x_ref[rows, :].astype(_F32)
        mean = jnp.mean(x, axis=-1, keepdims=True)
        xc = x - mean
        var = jnp.mean(xc * xc, axis=-1, keepdims=True)
        mean_b = _bf16_round(mean)
        var_b = _bf16_round(var)
        den = _bf16_round(jnp.sqrt(_bf16_round(var_b + _EPS)))
        d = _bf16_round(x - mean_b)
        xn = _bf16_round(d / den)
        xn_ref[rows, :] = xn.astype(_BF16)
        xnp_ref[rows, :] = pltpu.bitcast(_pack_rows(xn), _BF16)
        r = jnp.sum(xn * wr, axis=-1, keepdims=True)
        r_ref[rows, :] = _bf16_round(r)
        return carry

    lax.fori_loop(0, n_ch, ln_chunk, 0)

    for i in range(1, len(w_pairs)):
        w_copy(i).start()
    w_copy(0).wait()

    wvt_ref[...] = wqkv_ref[:, 2 * _D:3 * _D].T
    qscale = (_DH ** -0.5) * _LOG2E

    def proj_chunk(c, carry):
        start = pl.multiple_of(c * _CH, _CH)
        xn = xn_ref[pl.ds(start, _CH), :]
        qk = jnp.dot(xn, wqkv_ref[:, 0:2 * _D], preferred_element_type=_F32)
        q_ref[pl.ds(start, _CH), :] = (qk[:, 0:_D] * qscale).astype(_BF16)
        k_ref[pl.ds(start + _W, _CH), :] = qk[:, _D:2 * _D].astype(_BF16)
        vt = lax.dot_general(wvt_ref[...], xnp_ref[pl.ds(start, _CH), :], _NT,
                             preferred_element_type=_F32)
        vt_ref[:, pl.ds(start + _W, _CH)] = vt.astype(_BF16)
        return carry

    lax.fori_loop(0, n_ch, proj_chunk, 0)

    rv = r_ref[...]
    rmax = jnp.max(rv, axis=0, keepdims=True)
    tok = lax.broadcasted_iota(jnp.int32, (_S, 1), 0)
    idx = jnp.min(jnp.where(rv == rmax, tok, _S))
    base = pl.multiple_of((idx // 16) * 16, 16)
    tile = xn_ref[pl.ds(base, 16), :]
    row16 = lax.broadcasted_iota(jnp.int32, (16, _D), 0)
    xsel = jnp.where(row16 == (idx - base), tile.astype(_F32), 0.0).astype(_BF16)
    for i in range(1, len(w_pairs)):
        w_copy(i).wait()
    gpre = _bf16_round(lax.dot_general(xsel, wgt_ref[...], _NT, preferred_element_type=_F32))
    gate = _bf16_round(gpre * jax.nn.sigmoid(gpre))
    up = _bf16_round(lax.dot_general(xsel, wut_ref[...], _NT, preferred_element_type=_F32))
    hmid = (gate * up).astype(_BF16)
    y = _bf16_round(jnp.dot(hmid, wd_ref[...], preferred_element_type=_F32))
    rsel = _bf16_round(jax.nn.sigmoid(rmax))
    y = _bf16_round(y * rsel)
    upd_ref[...] = jnp.sum(y, axis=0, keepdims=True)

    head_u = lax.broadcasted_iota(jnp.int32, (_QB // 2, 128), 1) // _DH
    lane_o = lax.broadcasted_iota(jnp.int32, (_QB, 128), 1)
    parity_even = ((lane_o // _DH) % 2) == 0
    e_row = lax.broadcasted_iota(jnp.int32, (_QB, 128), 0)
    e_col = lax.broadcasted_iota(jnp.int32, (_QB, 128), 1) % _QB
    top_ok = e_row > e_col
    out_row = lax.broadcasted_iota(jnp.int32, (_SB, _D), 0)

    def first_row(q_start, half):
        if isinstance(q_start, int):
            return max(_W - (q_start + half * _QB), 0)
        return 0

    def stage_a(q_start, g, slot):
        lanes = slice(g * 128, (g + 1) * 128)
        for half in range(2):
            r_lo = first_row(q_start, half)
            q0 = q_start + half * _QB
            q0 = q0 if isinstance(q0, int) else pl.multiple_of(q0, _QB)
            kw = k_ref[pl.ds(q0 + r_lo, _KW - r_lo), lanes]
            qtu = pltpu.bitcast(q_ref[pl.ds(q0, _QB), lanes], _U32)
            order = [0, 1, 2, 3, 4, 5, 6, 7] if half == 0 else [1, 0, 3, 2, 5, 4, 7, 6]
            qmod = pltpu.bitcast(
                jnp.concatenate([jnp.where(head_u == h, qtu, jnp.zeros_like(qtu)) for h in order],
                                axis=0), _BF16)
            st = lax.dot_general(kw, qmod, _NT, preferred_element_type=_F32)
            n = _KW - r_lo
            cols = []
            for j in range(4):
                sj = st[:, 128 * j:128 * (j + 1)]
                parts = []
                if r_lo == 0:
                    parts.append(jnp.where(top_ok, sj[0:_QB], _NEG))
                    parts.append(sj[_QB:n - _QB])
                elif n > _QB:
                    parts.append(sj[0:n - _QB])
                parts.append(jnp.where(top_ok, _NEG, sj[n - _QB:n]))
                cols.append(jnp.concatenate(parts, axis=0))
            st = jnp.concatenate(cols, axis=1)
            st_ref[2 * slot + half, r_lo:_KW, :] = st
            m_ref[2 * slot + half] = jnp.max(st, axis=0, keepdims=True)

    def stage_b(q_start, g, slot):
        lanes = slice(g * 128, (g + 1) * 128)
        t0 = 0 if not isinstance(q_start, int) else max(_W - q_start, 0) // 128
        pads = []
        for half in range(2):
            r_lo = first_row(q_start, half)
            st = st_ref[2 * slot + half, r_lo:_KW, :]
            m = m_ref[2 * slot + half]
            pu = _pack_rows(jnp.exp2(st - m))
            n_top = (r_lo + _QB * half - 128 * t0) // 2
            n_bot = (_QB * (1 - half)) // 2
            parts = []
            if n_top:
                parts.append(jnp.zeros((n_top, 8 * _QB), _U32))
            parts.append(pu)
            if n_bot:
                parts.append(jnp.zeros((n_bot, 8 * _QB), _U32))
            pads.append(jnp.concatenate(parts, axis=0) if len(parts) > 1 else pu)
        nk = _SB + _W - 128 * t0
        qs = q_start + 128 * t0
        qs = qs if isinstance(qs, int) else pl.multiple_of(qs, _SB)
        vtw = vt_ref[lanes, pl.ds(qs, nk)]
        lo_k = lax.broadcasted_iota(jnp.int32, (nk // 2, 128), 1) < _QB
        ones_k = jnp.ones((_DH, nk), _BF16)
        raw = []
        for j in range(4):
            tl = slice(128 * j, 128 * (j + 1))
            e_t = pads[0][:, tl]
            o_t = pads[1][:, tl]
            ma = pltpu.bitcast(jnp.where(lo_k, e_t, o_t), _BF16)
            mb = pltpu.bitcast(jnp.where(lo_k, o_t, e_t), _BF16)
            for hh, mm in ((0, ma), (1, mb)):
                r0 = 32 * j + 16 * hh
                lhs = jnp.concatenate([vtw[r0:r0 + 16, :], ones_k], axis=0)
                raw.append(jnp.dot(lhs, mm, preferred_element_type=_F32))
        return raw

    def stage_f(raw, g):
        ot = [r[0:16, :] * (1.0 / r[16:17, :]) for r in raw]
        t = jnp.concatenate(ot, axis=0).T
        t_lo = t[0:_QB, :]
        t_hi = t[_QB:2 * _QB, :]
        o_e = jnp.where(parity_even, t_lo, t_hi)
        o_o = jnp.where(parity_even, t_hi, t_lo)
        oblk_ref[:, g * 128:(g + 1) * 128] = jnp.concatenate([o_e, o_o], axis=0).astype(_BF16)

    def stage_c(sb):
        q_start = pl.multiple_of(sb * _SB, _SB)
        attn = jnp.dot(oblk_ref[...], wo_ref[...], preferred_element_type=_F32)
        rows = pl.ds(q_start, _SB)
        res = x_ref[rows, :].astype(_F32) + attn + xn_ref[rows, :].astype(_F32)
        res = res + jnp.where(out_row == (idx - q_start), upd_ref[...], 0.0)
        o_ref[rows, :] = res.astype(o_ref.dtype)

    def super_block(sb, first):
        static = isinstance(sb, int)
        q_start = sb * _SB if static else pl.multiple_of(sb * _SB, _SB)
        pending = None
        for g in range(4):
            if g < 3:
                stage_a(q_start, g + 1, (g + 1) % 2)
            else:
                if static:
                    nxt = (sb + 1) * _SB
                else:
                    nxt = pl.multiple_of(jnp.minimum(sb + 1, n_sb - 1) * _SB, _SB)
                stage_a(nxt, 0, 0)
            if g == 0:
                if not first:
                    stage_f([res_ref[h] for h in range(8)], 3)
                    stage_c(sb - 1)
                    o_copy(sb - 1).start()
            else:
                stage_f(pending, g - 1)
            pending = stage_b(q_start, g, g % 2)
        for h in range(8):
            res_ref[h] = pending[h]

    def main_body(sb, carry):
        super_block(sb, False)
        return carry

    stage_a(0, 0, 0)
    super_block(0, True)
    super_block(1, False)
    lax.fori_loop(2, n_sb, main_body, 0)
    stage_f([res_ref[h] for h in range(8)], 3)
    stage_c(n_sb - 1)
    o_copy(n_sb - 1).start()
    for sb in range(n_sb):
        o_copy(sb).wait()


@jax.jit
def pallas_parallel_sum__sliding_block__moe_arch_mod__prompt_kernel(
    A_x: jax.Array,
    A_wqkv: jax.Array,
    A_wo: jax.Array,
    B_x: jax.Array,
    B_w_r: jax.Array,
    B_w_gate: jax.Array,
    B_w_up: jax.Array,
    B_w_down: jax.Array,
):
    del B_x
    B, S, D = A_x.shape
    any_spec = pl.BlockSpec(memory_space=pl.ANY)
    out = pl.pallas_call(
        _kernel,
        out_shape=jax.ShapeDtypeStruct((S, D), A_x.dtype),
        in_specs=[any_spec, any_spec, any_spec, pl.BlockSpec(memory_space=pltpu.VMEM),
                  any_spec, any_spec, any_spec],
        out_specs=any_spec,
        scratch_shapes=[
            pltpu.VMEM((_S, _D), _BF16),
            pltpu.VMEM((_D, 3 * _D), _BF16),
            pltpu.VMEM((_D, _D), _BF16),
            pltpu.VMEM((_F, _D), _BF16),
            pltpu.VMEM((_F, _D), _BF16),
            pltpu.VMEM((_F, _D), _BF16),
            pltpu.VMEM((_S, _D), _BF16),
            pltpu.VMEM((_S, _D), _BF16),
            pltpu.VMEM((_S, _D), _BF16),
            pltpu.VMEM((_S, _D), _BF16),
            pltpu.VMEM((_S + _W, _D), _BF16),
            pltpu.VMEM((_D, _S + _W), _BF16),
            pltpu.VMEM((_S, 1), _F32),
            pltpu.VMEM((_D, _D), _BF16),
            pltpu.VMEM((1, _D), _F32),
            pltpu.VMEM((4, _KW, 8 * _QB), _F32),
            pltpu.VMEM((4, 1, 8 * _QB), _F32),
            pltpu.VMEM((_SB, _D), _BF16),
            pltpu.VMEM((8, 2 * _DH, 128), _F32),
            pltpu.SemaphoreType.DMA((_S // _CH,)),
            pltpu.SemaphoreType.DMA((5,)),
            pltpu.SemaphoreType.DMA(()),
        ],
        compiler_params=pltpu.CompilerParams(vmem_limit_bytes=100 * 1024 * 1024),
        name="fused_ln_attn_moe",
    )(A_x.reshape(S, D), A_wqkv, A_wo, B_w_r, B_w_gate.T, B_w_up.T, B_w_down)
    return out.reshape(B, S, D)
```

```python
import jax
import jax.numpy as jnp
from jax import lax
import jax.experimental.pallas as pl
import jax.experimental.pallas.tpu as pltpu

_S = 2048
_D = 512
_DH = 16
_W = 256
_F = 1376
_EPS = 1e-5
_NEG = -1e9

_CH = 256
_QB = 64
_KW = _W + _QB
_SB = 128

_LOG2E = 1.4426950408889634
_F32 = jnp.float32
_BF16 = jnp.bfloat16
_U32 = jnp.uint32
_NT = (((1,), (1,)), ((), ()))


def _bf16_round(v):
    return v.astype(_BF16).astype(_F32)


def _pack_rows(a):
    r, c = a.shape
    a4 = a.reshape(r // 16, 2, 8, c)
    lo = a4[:, 0].reshape(r // 2, c)
    hi = a4[:, 1].reshape(r // 2, c)
    return pltpu.pack_elementwise([lo, hi], packed_dtype=_BF16)


def _kernel(x_hbm, wqkv_hbm, wo_hbm, wr_ref, wgt_hbm, wut_hbm, wd_hbm,
            o_hbm,
            x_ref, wqkv_ref, wo_ref, wgt_ref, wut_ref, wd_ref, o_ref,
            xn_ref, xnp_ref, q_ref, k_ref, vt_ref, r_ref, wvt_ref, upd_ref,
            st_ref, m_ref, oblk_ref, res_ref, sem_x, sem_w, sem_o):
    n_ch = _S // _CH
    n_sb = _S // _SB

    def x_copy(c):
        rows = pl.ds(pl.multiple_of(c * _CH, _CH), _CH)
        return pltpu.make_async_copy(x_hbm.at[rows, :], x_ref.at[rows, :], sem_x.at[c])

    w_pairs = ((wqkv_hbm, wqkv_ref), (wo_hbm, wo_ref), (wgt_hbm, wgt_ref),
               (wut_hbm, wut_ref), (wd_hbm, wd_ref))

    def w_copy(i):
        return pltpu.make_async_copy(w_pairs[i][0], w_pairs[i][1], sem_w.at[i])

    def o_copy(sb):
        rows = pl.ds(pl.multiple_of(sb * _SB, _SB), _SB)
        return pltpu.make_async_copy(o_ref.at[rows, :], o_hbm.at[rows, :], sem_o)

    x_copy(0).start()
    x_copy(1).start()
    w_copy(0).start()

    k_ref[0:_W, :] = jnp.zeros((_W, _D), _BF16)
    vt_ref[:, 0:_W] = jnp.zeros((_D, _W), _BF16)
    wr = wr_ref[...].reshape(1, _D).astype(_F32)

    def ln_rows(row0, nrows):
        rows = pl.ds(pl.multiple_of(row0, 16), nrows)
        x = x_ref[rows, :].astype(_F32)
        mean = jnp.mean(x, axis=-1, keepdims=True)
        xc = x - mean
        var = jnp.mean(xc * xc, axis=-1, keepdims=True)
        mean_b = _bf16_round(mean)
        var_b = _bf16_round(var)
        den = _bf16_round(jnp.sqrt(_bf16_round(var_b + _EPS)))
        d = _bf16_round(x - mean_b)
        xn = _bf16_round(d / den)
        xn_ref[rows, :] = xn.astype(_BF16)
        xnp_ref[rows, :] = pltpu.bitcast(_pack_rows(xn), _BF16)
        r = jnp.sum(xn * wr, axis=-1, keepdims=True)
        r_ref[rows, :] = _bf16_round(r)

    qscale = (_DH ** -0.5) * _LOG2E
    nsl = 256

    def proj_piece(c, i):
        start = pl.multiple_of(c * _CH, _CH)
        if i < 4:
            col = i * nsl
            xn = xn_ref[pl.ds(start, _CH), :]
            qk = jnp.dot(xn, wqkv_ref[:, col:col + nsl], preferred_element_type=_F32)
            if col < _D:
                q_ref[pl.ds(start, _CH), col:col + nsl] = (qk * qscale).astype(_BF16)
            else:
                k_ref[pl.ds(start + _W, _CH), col - _D:col - _D + nsl] = qk.astype(_BF16)
        else:
            f0 = (i - 4) * nsl
            vt = lax.dot_general(wvt_ref[f0:f0 + nsl, :], xnp_ref[pl.ds(start, _CH), :], _NT,
                                 preferred_element_type=_F32)
            vt_ref[f0:f0 + nsl, pl.ds(start + _W, _CH)] = vt.astype(_BF16)

    x_copy(0).wait()
    ln_rows(0, _CH)
    w_copy(0).wait()
    for c in range(2, n_ch):
        x_copy(c).start()
    for i in range(1, len(w_pairs)):
        w_copy(i).start()
    wvt_ref[...] = wqkv_ref[:, 2 * _D:3 * _D].T

    def lnproj_body(c, carry):
        x_copy(c + 1).wait()
        for i in range(6):
            proj_piece(c, i)
            if i >= 4:
                ln_rows((c + 1) * _CH + (i - 4) * (_CH // 2), _CH // 2)
        return carry

    lax.fori_loop(0, n_ch - 1, lnproj_body, 0)
    for i in range(6):
        proj_piece(n_ch - 1, i)

    rv = r_ref[...]
    rmax = jnp.max(rv, axis=0, keepdims=True)
    tok = lax.broadcasted_iota(jnp.int32, (_S, 1), 0)
    idx = jnp.min(jnp.where(rv == rmax, tok, _S))
    idx = jnp.minimum(idx, _S - 1)
    base = pl.multiple_of((idx // 16) * 16, 16)
    tile = xn_ref[pl.ds(base, 16), :]
    row16 = lax.broadcasted_iota(jnp.int32, (16, _D), 0)
    xsel = jnp.where(row16 == (idx - base), tile.astype(_F32), 0.0).astype(_BF16)
    for i in range(1, len(w_pairs)):
        w_copy(i).wait()
    gpre = _bf16_round(lax.dot_general(xsel, wgt_ref[...], _NT, preferred_element_type=_F32))
    gate = _bf16_round(gpre * jax.nn.sigmoid(gpre))
    up = _bf16_round(lax.dot_general(xsel, wut_ref[...], _NT, preferred_element_type=_F32))
    hmid = (gate * up).astype(_BF16)
    y = _bf16_round(jnp.dot(hmid, wd_ref[...], preferred_element_type=_F32))
    rsel = _bf16_round(jax.nn.sigmoid(rmax))
    y = _bf16_round(y * rsel)
    upd_ref[...] = jnp.sum(y, axis=0, keepdims=True)

    head_u = lax.broadcasted_iota(jnp.int32, (_QB // 2, 128), 1) // _DH
    lane_o = lax.broadcasted_iota(jnp.int32, (_QB, 128), 1)
    parity_even = ((lane_o // _DH) % 2) == 0
    e_row = lax.broadcasted_iota(jnp.int32, (_QB, 128), 0)
    e_col = lax.broadcasted_iota(jnp.int32, (_QB, 128), 1) % _QB
    top_ok = e_row > e_col
    out_row = lax.broadcasted_iota(jnp.int32, (_SB, _D), 0)

    def first_row(q_start, half):
        if isinstance(q_start, int):
            return max(_W - (q_start + half * _QB), 0)
        return 0

    def stage_a(q_start, g, slot):
        lanes = slice(g * 128, (g + 1) * 128)
        for half in range(2):
            r_lo = first_row(q_start, half)
            q0 = q_start + half * _QB
            q0 = q0 if isinstance(q0, int) else pl.multiple_of(q0, _QB)
            kw = k_ref[pl.ds(q0 + r_lo, _KW - r_lo), lanes]
            qtu = pltpu.bitcast(q_ref[pl.ds(q0, _QB), lanes], _U32)
            order = [0, 1, 2, 3, 4, 5, 6, 7] if half == 0 else [1, 0, 3, 2, 5, 4, 7, 6]
            qmod = pltpu.bitcast(
                jnp.concatenate([jnp.where(head_u == h, qtu, jnp.zeros_like(qtu)) for h in order],
                                axis=0), _BF16)
            st = lax.dot_general(kw, qmod, _NT, preferred_element_type=_F32)
            n = _KW - r_lo
            cols = []
            for j in range(4):
                sj = st[:, 128 * j:128 * (j + 1)]
                parts = []
                if r_lo == 0:
                    parts.append(jnp.where(top_ok, sj[0:_QB], _NEG))
                    parts.append(sj[_QB:n - _QB])
                elif n > _QB:
                    parts.append(sj[0:n - _QB])
                parts.append(jnp.where(top_ok, _NEG, sj[n - _QB:n]))
                cols.append(jnp.concatenate(parts, axis=0))
            st = jnp.concatenate(cols, axis=1)
            st_ref[2 * slot + half, r_lo:_KW, :] = st
            m_ref[2 * slot + half] = jnp.max(st, axis=0, keepdims=True)

    def stage_b(q_start, g, slot):
        lanes = slice(g * 128, (g + 1) * 128)
        t0 = 0 if not isinstance(q_start, int) else max(_W - q_start, 0) // 128
        pads = []
        for half in range(2):
            r_lo = first_row(q_start, half)
            st = st_ref[2 * slot + half, r_lo:_KW, :]
            m = m_ref[2 * slot + half]
            pu = _pack_rows(jnp.exp2(st - m))
            n_top = (r_lo + _QB * half - 128 * t0) // 2
            n_bot = (_QB * (1 - half)) // 2
            parts = []
            if n_top:
                parts.append(jnp.zeros((n_top, 8 * _QB), _U32))
            parts.append(pu)
            if n_bot:
                parts.append(jnp.zeros((n_bot, 8 * _QB), _U32))
            pads.append(jnp.concatenate(parts, axis=0) if len(parts) > 1 else pu)
        nk = _SB + _W - 128 * t0
        qs = q_start + 128 * t0
        qs = qs if isinstance(qs, int) else pl.multiple_of(qs, _SB)
        vtw = vt_ref[lanes, pl.ds(qs, nk)]
        lo_k = lax.broadcasted_iota(jnp.int32, (nk // 2, 128), 1) < _QB
        ones_k = jnp.ones((_DH, nk), _BF16)
        raw = []
        for j in range(4):
            tl = slice(128 * j, 128 * (j + 1))
            e_t = pads[0][:, tl]
            o_t = pads[1][:, tl]
            ma = pltpu.bitcast(jnp.where(lo_k, e_t, o_t), _BF16)
            mb = pltpu.bitcast(jnp.where(lo_k, o_t, e_t), _BF16)
            for hh, mm in ((0, ma), (1, mb)):
                r0 = 32 * j + 16 * hh
                lhs = jnp.concatenate([vtw[r0:r0 + 16, :], ones_k], axis=0)
                raw.append(jnp.dot(lhs, mm, preferred_element_type=_F32))
        return raw

    def stage_f(raw, g):
        ot = [r[0:16, :] * (1.0 / r[16:17, :]) for r in raw]
        t = jnp.concatenate(ot, axis=0).T
        t_lo = t[0:_QB, :]
        t_hi = t[_QB:2 * _QB, :]
        o_e = jnp.where(parity_even, t_lo, t_hi)
        o_o = jnp.where(parity_even, t_hi, t_lo)
        oblk_ref[:, g * 128:(g + 1) * 128] = jnp.concatenate([o_e, o_o], axis=0).astype(_BF16)

    def stage_c(sb):
        q_start = pl.multiple_of(sb * _SB, _SB)
        attn = jnp.dot(oblk_ref[...], wo_ref[...], preferred_element_type=_F32)
        rows = pl.ds(q_start, _SB)
        res = x_ref[rows, :].astype(_F32) + attn + xn_ref[rows, :].astype(_F32)
        res = res + jnp.where(out_row == (idx - q_start), upd_ref[...], 0.0)
        o_ref[rows, :] = res.astype(o_ref.dtype)

    def super_block(sb, first):
        static = isinstance(sb, int)
        q_start = sb * _SB if static else pl.multiple_of(sb * _SB, _SB)
        pending = None
        for g in range(4):
            if g < 3:
                stage_a(q_start, g + 1, (g + 1) % 2)
            else:
                if static:
                    nxt = (sb + 1) * _SB
                else:
                    nxt = pl.multiple_of(jnp.minimum(sb + 1, n_sb - 1) * _SB, _SB)
                stage_a(nxt, 0, 0)
            if g == 0:
                if not first:
                    stage_f([res_ref[h] for h in range(8)], 3)
                    stage_c(sb - 1)
                    o_copy(sb - 1).start()
            else:
                stage_f(pending, g - 1)
            pending = stage_b(q_start, g, g % 2)
        for h in range(8):
            res_ref[h] = pending[h]

    def main_body(i, carry):
        super_block(2 * i, False)
        super_block(2 * i + 1, False)
        return carry

    stage_a(0, 0, 0)
    super_block(0, True)
    super_block(1, False)
    lax.fori_loop(1, n_sb // 2, main_body, 0)
    stage_f([res_ref[h] for h in range(8)], 3)
    stage_c(n_sb - 1)
    o_copy(n_sb - 1).start()
    for sb in range(n_sb):
        o_copy(sb).wait()


@jax.jit
def pallas_parallel_sum__sliding_block__moe_arch_mod__prompt_kernel(
    A_x: jax.Array,
    A_wqkv: jax.Array,
    A_wo: jax.Array,
    B_x: jax.Array,
    B_w_r: jax.Array,
    B_w_gate: jax.Array,
    B_w_up: jax.Array,
    B_w_down: jax.Array,
):
    del B_x
    B, S, D = A_x.shape
    any_spec = pl.BlockSpec(memory_space=pl.ANY)
    out = pl.pallas_call(
        _kernel,
        out_shape=jax.ShapeDtypeStruct((S, D), A_x.dtype),
        in_specs=[any_spec, any_spec, any_spec, pl.BlockSpec(memory_space=pltpu.VMEM),
                  any_spec, any_spec, any_spec],
        out_specs=any_spec,
        scratch_shapes=[
            pltpu.VMEM((_S, _D), _BF16),
            pltpu.VMEM((_D, 3 * _D), _BF16),
            pltpu.VMEM((_D, _D), _BF16),
            pltpu.VMEM((_F, _D), _BF16),
            pltpu.VMEM((_F, _D), _BF16),
            pltpu.VMEM((_F, _D), _BF16),
            pltpu.VMEM((_S, _D), _BF16),
            pltpu.VMEM((_S, _D), _BF16),
            pltpu.VMEM((_S, _D), _BF16),
            pltpu.VMEM((_S, _D), _BF16),
            pltpu.VMEM((_S + _W, _D), _BF16),
            pltpu.VMEM((_D, _S + _W), _BF16),
            pltpu.VMEM((_S, 1), _F32),
            pltpu.VMEM((_D, _D), _BF16),
            pltpu.VMEM((1, _D), _F32),
            pltpu.VMEM((4, _KW, 8 * _QB), _F32),
            pltpu.VMEM((4, 1, 8 * _QB), _F32),
            pltpu.VMEM((_SB, _D), _BF16),
            pltpu.VMEM((8, 2 * _DH, 128), _F32),
            pltpu.SemaphoreType.DMA((_S // _CH,)),
            pltpu.SemaphoreType.DMA((5,)),
            pltpu.SemaphoreType.DMA(()),
        ],
        compiler_params=pltpu.CompilerParams(vmem_limit_bytes=100 * 1024 * 1024),
        name="fused_ln_attn_moe",
    )(A_x.reshape(S, D), A_wqkv, A_wo, B_w_r, B_w_gate.T, B_w_up.T, B_w_down)
    return out.reshape(B, S, D)
```
